```python
import jax
import jax.numpy as jnp

def _softmax(x, axis=-1):
    return jax.nn.softmax(x, axis=axis)
def _gelu(x):
    return jax.nn.gelu(x, approximate=True)
def _silu(x):
    return jax.nn.silu(x)
def _sigmoid(x):
    return jax.nn.sigmoid(x)
def _layernorm(x, axis=-1, eps=1e-5):
    m = jnp.mean(x, axis=axis, keepdims=True)
    v = jnp.var(x, axis=axis, keepdims=True)
    return (x - m) / jnp.sqrt(v + eps)
def _scatter_add(tgt, idx, src, axis=0):
    return tgt.at[idx].add(src)
def _segment_sum(src, seg, n):
    return jax.ops.segment_sum(src, seg, n)
class _Rng:
    def __init__(self, key):
        self._k = key
    def _next(self):
        self._k, sub = jax.random.split(self._k)
        return sub
    def normal(self, shape):
        return jax.random.normal(self._next(), shape, dtype=jnp.bfloat16)
    def randint(self, lo, hi, shape):
        return jax.random.randint(self._next(), shape, lo, hi, dtype=jnp.int32)
    def uniform(self, shape, lo=0.0, hi=1.0):
        return jax.random.uniform(self._next(), shape, jnp.bfloat16, lo, hi)
    def permutation(self, n):
        return jax.random.permutation(self._next(), n)


kernel_name = 'gated_mix__mha_block_cached__compressed_kv_cla__decode'

def setup_inputs():
    _rng = _Rng(jax.random.key(int.from_bytes(__import__("os").urandom(4), "little")))
    _w = (lambda a: (lambda t: t.astype(jnp.bfloat16) if jnp.issubdtype(t.dtype, jnp.floating) else t)(jnp.asarray(a)))
    def _A_setup():
        B, Sq, D = 2, 1, 512
        H, Sk, Dh = 32, 8192, 128
        return {
            "x": _w((lambda *s: _rng.normal(s) * 0.05)(B, Sq, D)),
            "k_cache": _w((lambda *s: _rng.normal(s) * 0.05)(B, H, Sk, Dh)),
            "v_cache": _w((lambda *s: _rng.normal(s) * 0.05)(B, H, Sk, Dh)),
            "wq": _w((lambda *s: _rng.normal(s) * 0.05)(D, H * Dh) * (D ** -0.5)),
            "wo": _w((lambda *s: _rng.normal(s) * 0.05)(H * Dh, D) * ((H * Dh) ** -0.5)),
        }
    _A_in = _A_setup()

    def _B_setup():
        B, H, Sq, Sk, D, M = 2, 32, 1, 8192, 128, 512
        Dc = 4 * D
        return {
            "x": _w((lambda *s: _rng.normal(s) * 0.05)(B, Sq, M)),
            "c_kv": _w((lambda *s: _rng.normal(s) * 0.05)(B, Sk, Dc)),
            "w_q": _w((lambda *s: _rng.normal(s) * 0.05)(M, H, D) * (M ** -0.5)),
            "w_uk": _w((lambda *s: _rng.normal(s) * 0.05)(Dc, H, D) * (Dc ** -0.5)),
            "w_uv": _w((lambda *s: _rng.normal(s) * 0.05)(Dc, H, D) * (Dc ** -0.5)),
            "w_o": _w((lambda *s: _rng.normal(s) * 0.05)(H, D, M) * ((H * D) ** -0.5)),
        }
    _B_in = _B_setup()

    return {
        "A_x": _A_in["x"],
        "A_k_cache": _A_in["k_cache"],
        "A_v_cache": _A_in["v_cache"],
        "A_wq": _A_in["wq"],
        "A_wo": _A_in["wo"],
        "B_x": _B_in["x"],
        "B_c_kv": _B_in["c_kv"],
        "B_w_q": _B_in["w_q"],
        "B_w_uk": _B_in["w_uk"],
        "B_w_uv": _B_in["w_uv"],
        "B_w_o": _B_in["w_o"],
        "gate_w": _w((lambda *s: _rng.normal(s) * 0.05)(512)),
    }

def reference(A_x, A_k_cache, A_v_cache, A_wq, A_wo, B_x, B_c_kv, B_w_q, B_w_uk, B_w_uv, B_w_o, gate_w):
    def _A_ref(x, k_cache, v_cache, wq, wo):
        B, Sq, D = x.shape
        H, Dh = 32, 128
        q = (lambda x, *d: x.transpose(*d))((x @ wq).reshape(B, Sq, H, Dh), 0, 2, 1, 3)
        scores = jnp.einsum("bhqd,bhkd->bhqk", q, k_cache) * (Dh ** -0.5)
        p = _softmax(scores, axis=-1)
        o = jnp.einsum("bhqk,bhkd->bhqd", p, v_cache)
        return (lambda x, *d: x.transpose(*d))(o, 0, 2, 1, 3).reshape(B, Sq, H * Dh) @ wo

    def _B_ref(x, c_kv, w_q, w_uk, w_uv, w_o):
        B, Sq, M = x.shape[0], x.shape[1], x.shape[2]
        Sk = c_kv.shape[1]
        H, D = w_q.shape[1], w_q.shape[2]
        q = jnp.einsum("bqm,mhd->bhqd", x, w_q)
        k = jnp.einsum("bkc,chd->bhkd", c_kv, w_uk)
        v = jnp.einsum("bkc,chd->bhkd", c_kv, w_uv)
        scores = jnp.einsum("bhqd,bhkd->bhqk", q, k) * (D ** -0.5)
        off = Sk - Sq
        qi = jnp.arange(Sq)[:, None]
        kj = jnp.arange(Sk)[None, :]
        cmask = kj <= (qi + off)
        scores = jnp.where(cmask[None, None], scores, -1e9)
        p = _softmax(scores, axis=-1)
        ctx = jnp.einsum("bhqk,bhkd->bhqd", p, v)
        return jnp.einsum("bhqd,hdm->bqm", ctx, w_o)

    x = A_x
    g = _sigmoid((x * gate_w).sum(-1, keepdims=True))
    a = _A_ref(x, A_k_cache, A_v_cache, A_wq, A_wo)
    b = _B_ref(x, B_c_kv, B_w_q, B_w_uk, B_w_uv, B_w_o)
    return g * a + (1 - g) * b
```

```python
import jax
import jax.numpy as jnp
import jax.experimental.pallas as pl
import jax.experimental.pallas.tpu as pltpu

F32 = jnp.float32
BF16 = jnp.bfloat16
_NT = (((1,), (1,)), ((), ()))

B, H, SK, DH, DM = 2, 32, 8192, 128, 512
DC = 4 * DH
NHEAD = B * H
CH = 4096
NCH = SK // CH
LOOK = 2
NSLOT = LOOK * 2 * NCH
WROWS = 4096
CROWS = 1024
J_WQ, J_UK, J_CKV, J_UV, J_WO, J_END = 0, 4, 8, 24, 28, 32
NSEM = 4
PIECE_BYTES = 32 * 1024


class _SplitCopy:
    def __init__(self, src, dst, rows, row_bytes, sem):
        self.src, self.dst, self.rows, self.sem = src, dst, rows, sem
        self.piece = PIECE_BYTES // row_bytes

    def start(self):
        half = self.rows // 2
        for o in range(0, half, self.piece):
            for t in range(2):
                sl = pl.ds(t * half + o, self.piece)
                pltpu.make_async_copy(self.src.at[sl], self.dst.at[sl],
                                      self.sem).start(priority=t)

    def wait(self):
        pltpu.make_async_copy(self.dst, self.dst, self.sem).wait()


def _dot(a, b):
    return jnp.dot(a, b, preferred_element_type=F32)


def _dot_nt(a, b):
    return jax.lax.dot_general(a, b, _NT, preferred_element_type=F32)


def _kernel(x_hbm, k_hbm, v_hbm, wq_hbm, wo_hbm, ckv_hbm, bwq_hbm, bwuk_hbm,
            bwuv_hbm, bwo_hbm, gw_hbm, o_ref,
            x_buf, gw_buf, wq_buf, wo_buf, ckv_buf, bwq_buf, bwuk_buf,
            bwuv_buf, bwo_buf, ring,
            q_scr, s_scr, p_scr, acca_scr, xcol_scr, qb_acc, qb_scr, qabs_scr,
            mb_scr, lb_scr, accb_scr, cc_scr, e0_scr, ctx_scr, outb_scr,
            kv_sems, b_sems, wo_sems, misc_sems):
    scale = DH ** -0.5

    def kv_copy(j, c):
        src = k_hbm if c < NCH else v_hbm
        slot = (j % LOOK) * (2 * NCH) + c
        return _SplitCopy(src.at[j, pl.ds((c % NCH) * CH, CH)], ring.at[slot], CH,
                          DH * 2, kv_sems.at[slot])

    def _rows_copy(hbm, buf, i, nrows, row_bytes, sem):
        rows = pl.ds(pl.multiple_of(i * nrows, nrows), nrows)
        return _SplitCopy(hbm.at[rows], buf.at[rows], nrows, row_bytes, sem)

    def wo_copy(i):
        return _rows_copy(wo_hbm, wo_buf, i, CROWS, DM * 2, wo_sems.at[i])

    def w_piece(hbm, buf, i, j):
        return _rows_copy(hbm, buf, i, WROWS, DH * 2, b_sems.at[j % NSEM])

    def c_piece(i, j):
        return _rows_copy(ckv_hbm, ckv_buf, i, CROWS, DC * 2, b_sems.at[j % NSEM])

    def o_piece(i, j):
        return _rows_copy(bwo_hbm, bwo_buf, i, CROWS, DM * 2, b_sems.at[j % NSEM])

    def b_piece_do(j, fn):
        if isinstance(j, int):
            if j < J_UK:
                fn(w_piece(bwq_hbm, bwq_buf, j - J_WQ, j))
            elif j < J_CKV:
                fn(w_piece(bwuk_hbm, bwuk_buf, j - J_UK, j))
            elif j < J_UV:
                fn(c_piece(j - J_CKV, j))
            elif j < J_WO:
                fn(w_piece(bwuv_hbm, bwuv_buf, j - J_UV, j))
            elif j < J_END:
                fn(o_piece(j - J_WO, j))
            return

        @pl.when(j < J_UK)
        def _():
            fn(w_piece(bwq_hbm, bwq_buf, j - J_WQ, j))

        @pl.when((j >= J_UK) & (j < J_CKV))
        def _():
            fn(w_piece(bwuk_hbm, bwuk_buf, j - J_UK, j))

        @pl.when((j >= J_CKV) & (j < J_UV))
        def _():
            fn(c_piece(j - J_CKV, j))

        @pl.when((j >= J_UV) & (j < J_WO))
        def _():
            fn(w_piece(bwuv_hbm, bwuv_buf, j - J_UV, j))

        @pl.when((j >= J_WO) & (j < J_END))
        def _():
            fn(o_piece(j - J_WO, j))

    start = lambda c: c.start()

    x_cp = pltpu.make_async_copy(x_hbm, x_buf, misc_sems.at[0])
    gw_cp = pltpu.make_async_copy(gw_hbm, gw_buf, misc_sems.at[1])
    x_cp.start()
    gw_cp.start()
    for r in range(0, DM // 2, 16):
        for c in range(0, H * DH, 1024):
            for t in range(2):
                sl = (pl.ds(t * (DM // 2) + r, 16), pl.ds(c, 1024))
                pltpu.make_async_copy(wq_hbm.at[sl], wq_buf.at[sl],
                                      misc_sems.at[2]).start(priority=t)
    wq_cp = pltpu.make_async_copy(wq_buf, wq_buf, misc_sems.at[2])
    for j in range(LOOK):
        for c in range(2 * NCH):
            kv_copy(j, c).start()
        if j == 0:
            wo_copy(0).start()
        b_piece_do(j, start)

    e_row = jax.lax.broadcasted_iota(jnp.int32, (128, WROWS), 0)
    e_col = jax.lax.broadcasted_iota(jnp.int32, (128, WROWS), 1)
    e0_scr[...] = jnp.where(e_col // H == e_row, 1.0, 0.0).astype(BF16)
    acca_scr[...] = jnp.zeros_like(acca_scr)
    qb_acc[...] = jnp.zeros_like(qb_acc)
    mb_scr[...] = jnp.full_like(mb_scr, -jnp.inf)
    lb_scr[...] = jnp.zeros_like(lb_scr)
    accb_scr[...] = jnp.zeros_like(accb_scr)
    ctx_scr[...] = jnp.zeros_like(ctx_scr)
    outb_scr[...] = jnp.zeros_like(outb_scr)

    x_cp.wait()
    gw_cp.wait()
    x0 = x_buf[0:1, :].astype(F32)
    x1 = x_buf[1:2, :].astype(F32)
    row8 = jax.lax.broadcasted_iota(jnp.int32, (8, DM), 0)
    x8 = jnp.where(row8 == 0, x0, jnp.where(row8 == 1, x1, 0.0))
    gate = jax.nn.sigmoid(
        jnp.sum(x8 * gw_buf[...].astype(F32).reshape(1, DM), axis=-1, keepdims=True))
    xcol_scr[0] = jnp.broadcast_to(x0, (128, DM)).T
    xcol_scr[1] = jnp.broadcast_to(x1, (128, DM)).T

    wq_cp.wait()
    x8b = x8.astype(BF16)
    for h in range(H):
        q_scr[h] = _dot(x8b, wq_buf[:, h * DH:(h + 1) * DH]).astype(BF16)

    def head_mask(shape):
        r = jax.lax.broadcasted_iota(jnp.int32, shape, 0)
        c = jax.lax.broadcasted_iota(jnp.int32, shape, 1)
        return r, c

    def phase_wq(j):
        base = j * (WROWS // H)

        def body(m, carry):
            a0, a1 = carry
            w = bwq_buf[pl.ds(pl.multiple_of((base + m) * H, H), H), :].astype(F32)
            a0 = a0 + w * xcol_scr[0, pl.ds(base + m, 1), :]
            a1 = a1 + w * xcol_scr[1, pl.ds(base + m, 1), :]
            return a0, a1

        a0, a1 = jax.lax.fori_loop(0, WROWS // H, body,
                                   (qb_acc[0:H, :], qb_acc[H:2 * H, :]), unroll=8)
        qb_acc[0:H, :] = a0
        qb_acc[H:2 * H, :] = a1

    def phase_uk(j):
        i = j - J_UK
        rows = pl.ds(pl.multiple_of(i * WROWS, WROWS), WROWS)
        qb = qb_acc[...].astype(BF16)
        r = _dot_nt(bwuk_buf[rows, :], qb)
        rr, cc = head_mask((H, 128))
        keep = rr == (cc % H)
        r3 = jnp.where(keep[None], r.reshape(WROWS // H, H, 128), 0.0)
        qat = jnp.sum(r3, axis=1)
        qabs_scr[i] = qat.T.astype(BF16)

    def phase_ckv(j):
        i = j - J_CKV
        b = i // (SK // CROWS)
        rows = pl.ds(pl.multiple_of(i * CROWS, CROWS), CROWS)
        hrows = pl.ds(pl.multiple_of(b * H, H), H)
        s = jnp.zeros((H, CROWS), F32)
        for t in range(DC // 128):
            s = s + _dot_nt(qabs_scr[t, hrows, :], ckv_buf[rows, t * 128:(t + 1) * 128])
        m_old = mb_scr[hrows, :]
        m_new = jnp.maximum(m_old, jnp.max(s, axis=-1, keepdims=True))
        alpha = jnp.exp((m_old - m_new) * scale)
        p = jnp.exp((s - m_new) * scale)
        lb_scr[hrows, :] = lb_scr[hrows, :] * alpha + jnp.sum(p, axis=-1, keepdims=True)
        accb_scr[hrows, :] = accb_scr[hrows, :] * alpha + _dot(p.astype(BF16), ckv_buf[rows, :])
        mb_scr[hrows, :] = m_new

    def phase_uv(j):
        i = j - J_UV
        rows = pl.ds(pl.multiple_of(i * WROWS, WROWS), WROWS)

        @pl.when(i == 0)
        def _():
            cc = (accb_scr[...] / lb_scr[...]).astype(BF16)
            for t in range(DC // 128):
                cc_scr[t] = cc[:, t * 128:(t + 1) * 128]

        z = _dot(cc_scr[i], e0_scr[...])
        rr, cc = head_mask((2 * H, WROWS))
        z = jnp.where((rr % H) == (cc % H), z, 0.0).astype(BF16)
        ctx_scr[...] += _dot(z, bwuv_buf[rows, :])

    def phase_wo(j):
        i = j - J_WO
        rows = pl.ds(pl.multiple_of(i * CROWS, CROWS), CROWS)
        nh = CROWS // DH
        ctx = ctx_scr[...]
        lhs = jnp.concatenate([ctx] * nh, axis=1)
        rr, cc = head_mask((2 * H, CROWS))
        lhs = jnp.where((rr % H) == (cc // DH + i * nh), lhs, 0.0).astype(BF16)
        outb_scr[...] += _dot(lhs, bwo_buf[rows, :])

    def head_body(j, carry):
        b = j // H
        h = j % H
        par = j % LOOK
        more = j + LOOK < NHEAD
        q = q_scr[h]
        for c in range(NCH):
            kv_copy(j, c).wait()
            s_scr[:, c * CH:(c + 1) * CH] = _dot_nt(q, ring[par * 2 * NCH + c])

            @pl.when(more)
            def _():
                kv_copy(j + LOOK, c).start()

        s = s_scr[...]
        m = jnp.max(s, axis=-1, keepdims=True)
        p = jnp.exp((s - m) * scale)
        l = jnp.sum(p, axis=-1, keepdims=True)
        p_scr[...] = p.astype(BF16)
        acc = jnp.zeros((8, DH), F32)
        for c in range(NCH):
            kv_copy(j, NCH + c).wait()
            acc = acc + _dot(p_scr[:, c * CH:(c + 1) * CH], ring[par * 2 * NCH + NCH + c])

            @pl.when(more)
            def _():
                kv_copy(j + LOOK, NCH + c).start()

        @pl.when(j + LOOK < J_END)
        def _():
            b_piece_do(j + LOOK, start)

        hpp = CROWS // DH

        @pl.when((j + LOOK < H) & ((j + LOOK) % hpp == 0))
        def _():
            wo_copy((j + LOOK) // hpp).start()

        @pl.when((j < H) & (j % hpp == 0))
        def _():
            wo_copy(j // hpp).wait()

        r8 = jax.lax.broadcasted_iota(jnp.int32, (8, DH), 0)
        o = jnp.where(r8 == b, acc / l, 0.0).astype(BF16)
        hr = pl.ds(pl.multiple_of(h * DH, DH), DH)
        acca_scr[...] += _dot(o, wo_buf[hr, :])

        @pl.when(j < J_END)
        def _():
            b_piece_do(j, lambda c: c.wait())

        @pl.when(j < J_UK)
        def _():
            phase_wq(j)

        @pl.when((j >= J_UK) & (j < J_CKV))
        def _():
            phase_uk(j)

        @pl.when((j >= J_CKV) & (j < J_UV))
        def _():
            phase_ckv(j)

        @pl.when((j >= J_UV) & (j < J_WO))
        def _():
            phase_uv(j)

        @pl.when((j >= J_WO) & (j < J_END))
        def _():
            phase_wo(j)

        return carry

    jax.lax.fori_loop(0, NHEAD, head_body, 0)

    ob = outb_scr[...]
    ob0 = jnp.sum(ob[0:H], axis=0, keepdims=True)
    ob1 = jnp.sum(ob[H:2 * H], axis=0, keepdims=True)
    outb = jnp.where(row8 == 0, ob0, jnp.where(row8 == 1, ob1, 0.0))
    res = (gate * acca_scr[...] + (1.0 - gate) * outb).astype(BF16)
    o_ref[...] = res[0:B]


@jax.jit
def pallas_gated_mix__mha_block_cached__compressed_kv_cla__decode_kernel(
    A_x: jax.Array,
    A_k_cache: jax.Array,
    A_v_cache: jax.Array,
    A_wq: jax.Array,
    A_wo: jax.Array,
    B_x: jax.Array,
    B_c_kv: jax.Array,
    B_w_q: jax.Array,
    B_w_uk: jax.Array,
    B_w_uv: jax.Array,
    B_w_o: jax.Array,
    gate_w: jax.Array,
):
    del B_x
    k = A_k_cache.reshape(NHEAD, SK, DH)
    v = A_v_cache.reshape(NHEAD, SK, DH)
    ckv = B_c_kv.reshape(B * SK, DC)
    bwq = B_w_q.reshape(DM * H, DH)
    bwuk = B_w_uk.reshape(DC * H, DH)
    bwuv = B_w_uv.reshape(DC * H, DH)
    bwo = B_w_o.reshape(H * DH, DM)

    any_spec = pl.BlockSpec(memory_space=pl.ANY)
    scratch = [
        pltpu.VMEM((B, DM), BF16),
        pltpu.VMEM((DM,), BF16),
        pltpu.VMEM((DM, H * DH), BF16),
        pltpu.VMEM((H * DH, DM), BF16),
        pltpu.VMEM((B * SK, DC), BF16),
        pltpu.VMEM((DM * H, DH), BF16),
        pltpu.VMEM((DC * H, DH), BF16),
        pltpu.VMEM((DC * H, DH), BF16),
        pltpu.VMEM((H * DH, DM), BF16),
        pltpu.VMEM((NSLOT, CH, DH), BF16),
        pltpu.VMEM((H, 8, DH), BF16),
        pltpu.VMEM((8, SK), F32),
        pltpu.VMEM((8, SK), BF16),
        pltpu.VMEM((8, DM), F32),
        pltpu.VMEM((B, DM, 128), F32),
        pltpu.VMEM((128, DH), F32),
        pltpu.VMEM((128, DH), BF16),
        pltpu.VMEM((DC // 128, 128, 128), BF16),
        pltpu.VMEM((2 * H, 1), F32),
        pltpu.VMEM((2 * H, 1), F32),
        pltpu.VMEM((2 * H, DC), F32),
        pltpu.VMEM((DC // 128, 2 * H, 128), BF16),
        pltpu.VMEM((128, WROWS), BF16),
        pltpu.VMEM((2 * H, DH), F32),
        pltpu.VMEM((2 * H, DM), F32),
        pltpu.SemaphoreType.DMA((NSLOT,)),
        pltpu.SemaphoreType.DMA((NSEM,)),
        pltpu.SemaphoreType.DMA((NSEM,)),
        pltpu.SemaphoreType.DMA((3,)),
    ]
    out = pl.pallas_call(
        _kernel,
        in_specs=[any_spec] * 11,
        out_specs=pl.BlockSpec(memory_space=pltpu.VMEM),
        out_shape=jax.ShapeDtypeStruct((B, DM), BF16),
        scratch_shapes=scratch,
        compiler_params=pltpu.CompilerParams(vmem_limit_bytes=100 * 1024 * 1024),
    )(A_x.reshape(B, DM), k, v, A_wq, A_wo, ckv, bwq, bwuk, bwuv, bwo, gate_w)
    return out.reshape(B, 1, DM)
```

```python
import jax
import jax.numpy as jnp
import jax.experimental.pallas as pl
import jax.experimental.pallas.tpu as pltpu

F32 = jnp.float32
BF16 = jnp.bfloat16
_NT = (((1,), (1,)), ((), ()))

B, H, SK, DH, DM = 2, 32, 8192, 128, 512
DC = 4 * DH
NHEAD = B * H
NCH = 4
CH = SK // NCH
KV_PIECE = 168
W_PIECE = 168
C_PIECE = 40
WROWS = 2048
CROWS = 512
P_CKV, P_UV, P_END = 8, 24, 32
J_UK, J_CKV, J_UV, J_WO, J_END = 8, 12, 32, 36, 40


def _dot(a, b):
    return jnp.dot(a, b, preferred_element_type=F32)


def _dot_nt(a, b):
    return jax.lax.dot_general(a, b, _NT, preferred_element_type=F32)


def _pieces(rows, piece):
    return [(o, min(piece, rows - o)) for o in range(0, rows, piece)]


def _start_pair(a, b, sem_a, sem_b):
    pa, pb = _pieces(a[2], a[3]), _pieces(b[2], b[3])
    for i in range(max(len(pa), len(pb))):
        for t, (cp, ps, sem) in enumerate(((a, pa, sem_a), (b, pb, sem_b))):
            if i < len(ps):
                sl = pl.ds(ps[i][0], ps[i][1])
                pltpu.make_async_copy(cp[0].at[sl], cp[1].at[sl], sem).start(priority=t)


def _start_split(src, dst, rows, piece, sem):
    half = rows // 2
    lo, hi = pl.ds(0, half), pl.ds(half, half)
    _start_pair((src.at[lo], dst.at[lo], half, piece), (src.at[hi], dst.at[hi], half, piece),
                sem, sem)


def _wait(dst, sem):
    pltpu.make_async_copy(dst, dst, sem).wait()


def _kernel(x_hbm, k_hbm, v_hbm, wq_hbm, wo_hbm, ckv_hbm, bwq_hbm, bwuk_hbm,
            bwuv_hbm, bwo_hbm, gw_hbm, o_ref,
            x_buf, gw_buf, wq_buf, wo_buf, ckv_buf, bwq_buf, bwuk_buf,
            bwuv_buf, bwo_buf, ring,
            s_scr, p_scr, acca_scr, xcol_scr, qb_acc, qabs_scr,
            mb_scr, lb_scr, accb_scr, cc_scr, e0_scr, ctx_scr, outb_scr,
            kv_sems, b_sems, misc_sems):
    scale = DH ** -0.5

    def k_cp(j, c):
        return (k_hbm.at[j, pl.ds(c * CH, CH)], ring.at[c, pl.ds(0, CH)], CH, KV_PIECE)

    def v_cp(j, c):
        return (v_hbm.at[j, pl.ds(c * CH, CH)], ring.at[c, pl.ds(CH, CH)], CH, KV_PIECE)

    def rows_cp(hbm, buf, start, nrows, piece):
        if not isinstance(start, int):
            start = pl.multiple_of(start, nrows)
        rows = pl.ds(start, nrows)
        return (hbm.at[rows], buf.at[rows], nrows, piece)

    def part_copies(kind, i):
        if kind == 0:
            return (rows_cp(bwq_hbm, bwq_buf, i * WROWS, WROWS, W_PIECE),
                    rows_cp(bwuk_hbm, bwuk_buf, i * WROWS, WROWS, W_PIECE))
        if kind == 1:
            i = i - P_CKV
            return (rows_cp(ckv_hbm, ckv_buf, i * CROWS, CROWS, C_PIECE),
                    rows_cp(ckv_hbm, ckv_buf, SK + i * CROWS, CROWS, C_PIECE))
        i = i - P_UV
        return (rows_cp(bwuv_hbm, bwuv_buf, i * WROWS, WROWS, W_PIECE),
                rows_cp(bwo_hbm, bwo_buf, i * CROWS, CROWS, C_PIECE))

    def part_do(i, fn):
        sa, sb = b_sems.at[0, i % 4], b_sems.at[1, i % 4]
        if isinstance(i, int):
            kind = 0 if i < P_CKV else (1 if i < P_UV else 2)
            fn(*part_copies(kind, i), sa, sb)
            return

        @pl.when(i < P_CKV)
        def _():
            fn(*part_copies(0, i), sa, sb)

        @pl.when((i >= P_CKV) & (i < P_UV))
        def _():
            fn(*part_copies(1, i), sa, sb)

        @pl.when((i >= P_UV) & (i < P_END))
        def _():
            fn(*part_copies(2, i), sa, sb)

    def part_wait(a, b, sa, sb):
        _wait(a[1], sa)
        _wait(b[1], sb)

    x_cp = pltpu.make_async_copy(x_hbm, x_buf, misc_sems.at[0])
    gw_cp = pltpu.make_async_copy(gw_hbm, gw_buf, misc_sems.at[1])
    x_cp.start()
    gw_cp.start()
    i = 0
    for r in range(0, DM, 16):
        for c in range(0, H * DH, 1024):
            sl = (pl.ds(r, 16), pl.ds(c, 1024))
            pltpu.make_async_copy(wq_hbm.at[sl], wq_buf.at[sl], misc_sems.at[2]).start(priority=0)
            sl = pl.ds(i * 32, 32)
            pltpu.make_async_copy(wo_hbm.at[sl], wo_buf.at[sl], misc_sems.at[3]).start(priority=1)
            i += 1
    for c in range(NCH):
        src, dst, rows, piece = k_cp(0, c)
        _start_split(src, dst, rows, piece, kv_sems.at[c])
    part_do(0, _start_pair)

    acca_scr[...] = jnp.zeros_like(acca_scr)
    qb_acc[...] = jnp.zeros_like(qb_acc)
    mb_scr[...] = jnp.full_like(mb_scr, -jnp.inf)
    lb_scr[...] = jnp.zeros_like(lb_scr)
    accb_scr[...] = jnp.zeros_like(accb_scr)
    ctx_scr[...] = jnp.zeros_like(ctx_scr)
    outb_scr[...] = jnp.zeros_like(outb_scr)

    x_cp.wait()
    gw_cp.wait()
    x0 = x_buf[0:1, :].astype(F32)
    x1 = x_buf[1:2, :].astype(F32)
    row8 = jax.lax.broadcasted_iota(jnp.int32, (8, DM), 0)
    x8 = jnp.where(row8 == 0, x0, jnp.where(row8 == 1, x1, 0.0))
    x8b = x8.astype(BF16)
    gate = jax.nn.sigmoid(
        jnp.sum(x8 * gw_buf[...].astype(F32).reshape(1, DM), axis=-1, keepdims=True))

    def q_of(h):
        cols = pl.ds(h * DH if isinstance(h, int) else pl.multiple_of(h * DH, DH), DH)
        return _dot(x8b, wq_buf[:, cols]).astype(BF16)

    def softmax():
        s = s_scr[...]
        m = jnp.max(s, axis=-1, keepdims=True)
        p = jnp.exp((s - m) * scale)
        p_scr[...] = p.astype(BF16)
        return jnp.sum(p, axis=-1, keepdims=True)

    def qk(q, c):
        s_scr[:, c * CH:(c + 1) * CH] = _dot_nt(q, ring[c, 0:CH, :])

    def pv(c):
        return _dot(p_scr[:, c * CH:(c + 1) * CH], ring[c, CH:2 * CH, :])

    def finalize(j, acc, l):
        b = j // H
        h = j % H
        r8 = jax.lax.broadcasted_iota(jnp.int32, (8, DH), 0)
        o = jnp.where(r8 == b, acc / l, 0.0).astype(BF16)
        hr = pl.ds(h * DH if isinstance(h, int) else pl.multiple_of(h * DH, DH), DH)
        acca_scr[...] += _dot(o, wo_buf[hr, :])

    def iota2(shape):
        return (jax.lax.broadcasted_iota(jnp.int32, shape, 0),
                jax.lax.broadcasted_iota(jnp.int32, shape, 1))

    def phase_wq(j):
        nm = WROWS // H
        base = j * nm

        @pl.when(j == 0)
        def _():
            xcol_scr[0] = jnp.broadcast_to(x0, (128, DM)).T
            xcol_scr[1] = jnp.broadcast_to(x1, (128, DM)).T

        def body(m, carry):
            a0, a1 = carry
            w = bwq_buf[pl.ds(pl.multiple_of((base + m) * H, H), H), :].astype(F32)
            a0 = a0 + w * xcol_scr[0, pl.ds(base + m, 1), :]
            a1 = a1 + w * xcol_scr[1, pl.ds(base + m, 1), :]
            return a0, a1

        a0, a1 = jax.lax.fori_loop(0, nm, body,
                                   (qb_acc[0:H, :], qb_acc[H:2 * H, :]), unroll=8)
        qb_acc[0:H, :] = a0
        qb_acc[H:2 * H, :] = a1

    def phase_uk(j):
        i = j - J_UK
        n = 128 * H
        rows = pl.ds(pl.multiple_of(i * n, n), n)
        qb = qb_acc[...].astype(BF16)
        r = _dot_nt(bwuk_buf[rows, :], qb)
        rr, cc = iota2((H, 128))
        keep = rr == (cc % H)
        r3 = jnp.where(keep[None], r.reshape(128, H, 128), 0.0)
        qat = jnp.sum(r3, axis=1)
        qabs_scr[i] = qat.T.astype(BF16)

    def phase_ckv(j):
        i = j - J_CKV
        for b in range(B):
            rows = pl.ds(pl.multiple_of(b * SK + i * CROWS, CROWS), CROWS)
            hrows = slice(b * H, (b + 1) * H)
            s = jnp.zeros((H, CROWS), F32)
            for t in range(DC // 128):
                s = s + _dot_nt(qabs_scr[t, hrows, :], ckv_buf[rows, t * 128:(t + 1) * 128])
            m_old = mb_scr[hrows, :]
            m_new = jnp.maximum(m_old, jnp.max(s, axis=-1, keepdims=True))
            alpha = jnp.exp((m_old - m_new) * scale)
            p = jnp.exp((s - m_new) * scale)
            lb_scr[hrows, :] = lb_scr[hrows, :] * alpha + jnp.sum(p, axis=-1, keepdims=True)
            accb_scr[hrows, :] = (accb_scr[hrows, :] * alpha
                                  + _dot(p.astype(BF16), ckv_buf[rows, :]))
            mb_scr[hrows, :] = m_new

    def phase_uv(j):
        i = j - J_UV
        n = 128 * H
        rows = pl.ds(pl.multiple_of(i * n, n), n)

        @pl.when(i == 0)
        def _():
            cc = (accb_scr[...] / lb_scr[...]).astype(BF16)
            for t in range(DC // 128):
                cc_scr[t] = cc[:, t * 128:(t + 1) * 128]
            e_row, e_col = iota2((128, n))
            e0_scr[...] = jnp.where(e_col // H == e_row, 1.0, 0.0).astype(BF16)

        z = _dot(cc_scr[i], e0_scr[...])
        rr, cc = iota2((2 * H, n))
        z = jnp.where((rr % H) == (cc % H), z, 0.0).astype(BF16)
        ctx_scr[...] += _dot(z, bwuv_buf[rows, :])

    def phase_wo(j):
        i = j - J_WO
        nh = 8
        n = nh * DH
        rows = pl.ds(pl.multiple_of(i * n, n), n)
        ctx = ctx_scr[...]
        lhs = jnp.concatenate([ctx] * nh, axis=1)
        rr, cc = iota2((2 * H, n))
        lhs = jnp.where((rr % H) == (cc // DH + i * nh), lhs, 0.0).astype(BF16)
        outb_scr[...] += _dot(lhs, bwo_buf[rows, :])

    _wait(wq_buf, misc_sems.at[2])
    q0 = q_of(0)
    for c in range(NCH):
        _wait(ring.at[c, pl.ds(0, CH)], kv_sems.at[c])
        qk(q0, c)
        _start_pair(k_cp(1, c), v_cp(0, c), kv_sems.at[c], kv_sems.at[c])
    l0 = softmax()
    _wait(wo_buf, misc_sems.at[3])

    def head_body(j, l):
        q = q_of((j + 1) % H)
        acc = jnp.zeros((8, DH), F32)
        for c in range(NCH):
            _wait(ring.at[c], kv_sems.at[c])
            qk(q, c)
            acc = acc + pv(c)

            @pl.when(j < NHEAD - 2)
            def _():
                _start_pair(k_cp(j + 2, c), v_cp(j + 1, c), kv_sems.at[c], kv_sems.at[c])

            @pl.when(j == NHEAD - 2)
            def _():
                src, dst, rows, piece = v_cp(NHEAD - 1, c)
                _start_split(src, dst, rows, piece, kv_sems.at[c])

        @pl.when(j + 1 < P_END)
        def _():
            part_do(j + 1, _start_pair)

        finalize(j, acc, l)
        l_next = softmax()

        @pl.when(j < P_END)
        def _():
            part_do(j, part_wait)

        @pl.when(j < J_UK)
        def _():
            phase_wq(j)

        @pl.when((j >= J_UK) & (j < J_CKV))
        def _():
            phase_uk(j)

        @pl.when((j >= J_CKV) & (j < J_CKV + 16))
        def _():
            phase_ckv(j)

        @pl.when((j >= J_UV) & (j < J_WO))
        def _():
            phase_uv(j)

        @pl.when((j >= J_WO) & (j < J_END))
        def _():
            phase_wo(j)

        return l_next

    l = jax.lax.fori_loop(0, NHEAD - 1, head_body, l0)

    ob = outb_scr[...]
    ob0 = jnp.sum(ob[0:H], axis=0, keepdims=True)
    ob1 = jnp.sum(ob[H:2 * H], axis=0, keepdims=True)
    outb = (1.0 - gate) * jnp.where(row8 == 0, ob0, jnp.where(row8 == 1, ob1, 0.0))

    acc = jnp.zeros((8, DH), F32)
    for c in range(NCH):
        _wait(ring.at[c, pl.ds(CH, CH)], kv_sems.at[c])
        acc = acc + pv(c)
    finalize(NHEAD - 1, acc, l)
    res = (gate * acca_scr[...] + outb).astype(BF16)
    o_ref[...] = res[0:B]


@jax.jit
def pallas_gated_mix__mha_block_cached__compressed_kv_cla__decode_kernel(
    A_x: jax.Array,
    A_k_cache: jax.Array,
    A_v_cache: jax.Array,
    A_wq: jax.Array,
    A_wo: jax.Array,
    B_x: jax.Array,
    B_c_kv: jax.Array,
    B_w_q: jax.Array,
    B_w_uk: jax.Array,
    B_w_uv: jax.Array,
    B_w_o: jax.Array,
    gate_w: jax.Array,
):
    del B_x
    k = A_k_cache.reshape(NHEAD, SK, DH)
    v = A_v_cache.reshape(NHEAD, SK, DH)
    ckv = B_c_kv.reshape(B * SK, DC)
    bwq = B_w_q.reshape(DM * H, DH)
    bwuk = B_w_uk.reshape(DC * H, DH)
    bwuv = B_w_uv.reshape(DC * H, DH)
    bwo = B_w_o.reshape(H * DH, DM)

    any_spec = pl.BlockSpec(memory_space=pl.ANY)
    scratch = [
        pltpu.VMEM((B, DM), BF16),
        pltpu.VMEM((DM,), BF16),
        pltpu.VMEM((DM, H * DH), BF16),
        pltpu.VMEM((H * DH, DM), BF16),
        pltpu.VMEM((B * SK, DC), BF16),
        pltpu.VMEM((DM * H, DH), BF16),
        pltpu.VMEM((DC * H, DH), BF16),
        pltpu.VMEM((DC * H, DH), BF16),
        pltpu.VMEM((H * DH, DM), BF16),
        pltpu.VMEM((NCH, 2 * CH, DH), BF16),
        pltpu.VMEM((8, SK), F32),
        pltpu.VMEM((8, SK), BF16),
        pltpu.VMEM((8, DM), F32),
        pltpu.VMEM((B, DM, 128), F32),
        pltpu.VMEM((128, DH), F32),
        pltpu.VMEM((DC // 128, 128, 128), BF16),
        pltpu.VMEM((2 * H, 1), F32),
        pltpu.VMEM((2 * H, 1), F32),
        pltpu.VMEM((2 * H, DC), F32),
        pltpu.VMEM((DC // 128, 2 * H, 128), BF16),
        pltpu.VMEM((128, 128 * H), BF16),
        pltpu.VMEM((2 * H, DH), F32),
        pltpu.VMEM((2 * H, DM), F32),
        pltpu.SemaphoreType.DMA((NCH,)),
        pltpu.SemaphoreType.DMA((2, 4)),
        pltpu.SemaphoreType.DMA((4,)),
    ]
    out = pl.pallas_call(
        _kernel,
        in_specs=[any_spec] * 11,
        out_specs=pl.BlockSpec(memory_space=pltpu.VMEM),
        out_shape=jax.ShapeDtypeStruct((B, DM), BF16),
        scratch_shapes=scratch,
        compiler_params=pltpu.CompilerParams(vmem_limit_bytes=100 * 1024 * 1024),
    )(A_x.reshape(B, DM), k, v, A_wq, A_wo, ckv, bwq, bwuk, bwuv, bwo, gate_w)
    return out.reshape(B, 1, DM)
```

```python
import jax
import jax.numpy as jnp
import jax.experimental.pallas as pl
import jax.experimental.pallas.tpu as pltpu

F32 = jnp.float32
BF16 = jnp.bfloat16
_NT = (((1,), (1,)), ((), ()))

B, H, SK, DH, DM = 2, 32, 8192, 128, 512
DC = 4 * DH
NHEAD = B * H
NCH = 4
CH = SK // NCH
NS = 8
N_PIECE = 160
C_PIECE = 40
WROWS = 2048
CROWS = 512
P_CKV, P_UV, P_END = 8, 24, 32
J_UK, J_CKV, J_UV, J_WO, J_END = 8, 12, 32, 36, 40
LATE0 = 28 * DH
LATE = ((0, 256), (256, 128), (384, 128))


def _dot(a, b):
    return jnp.dot(a, b, preferred_element_type=F32)


def _dot_nt(a, b):
    return jax.lax.dot_general(a, b, _NT, preferred_element_type=F32)


def _iota2(shape):
    return (jax.lax.broadcasted_iota(jnp.int32, shape, 0),
            jax.lax.broadcasted_iota(jnp.int32, shape, 1))


def _pieces(rows, piece):
    return [(o, min(piece, rows - o)) for o in range(0, rows, piece)]


def _start_pair(a, b, sem_a, sem_b):
    pa, pb = _pieces(a[2], a[3]), _pieces(b[2], b[3])
    for i in range(max(len(pa), len(pb))):
        for t, (cp, ps, sem) in enumerate(((a, pa, sem_a), (b, pb, sem_b))):
            if i < len(ps):
                sl = pl.ds(*ps[i])
                pltpu.make_async_copy(cp[0].at[sl], cp[1].at[sl], sem).start(priority=t)


def _halves(src, dst, rows, piece):
    half = rows // 2
    lo, hi = pl.ds(0, half), pl.ds(half, half)
    return ((src.at[lo], dst.at[lo], half, piece), (src.at[hi], dst.at[hi], half, piece))


def _wait(dst, sem):
    pltpu.make_async_copy(dst, dst, sem).wait()


def _kernel(x_hbm, k_hbm, v_hbm, wq_hbm, wo_hbm, ckv_hbm, bwq_hbm, bwuk_hbm,
            bwuv_hbm, bwo_hbm, gw_hbm, o_ref,
            x_buf, gw_buf, wq_buf, wo_buf, ckv_buf, bwq_buf, bwuk_buf,
            bwuv_buf, bwo_buf, ring,
            s_scr, p_scr, acca_scr, xcol_scr, qb_acc, qabs_scr,
            mb_scr, lb_scr, accb_scr, cc_scr, e0_scr, ctx_scr, outb_scr,
            kv_sems, b_sems, misc_sems, late_sems):
    scale = DH ** -0.5

    def slot_of(j, c):
        return (NCH * (j + 1) + c) % NS

    def k_cp(j, c, slot):
        return (k_hbm.at[j, pl.ds(c * CH, CH)], ring.at[slot, pl.ds(0, CH)], CH, N_PIECE)

    def v_cp(j, c, slot):
        return (v_hbm.at[j, pl.ds(c * CH, CH)], ring.at[slot, pl.ds(CH, CH)], CH, N_PIECE)

    def issue_pair(j, c, slot):
        sem = kv_sems.at[slot]
        _start_pair(k_cp(j + 1, c, slot), v_cp(j, c, slot), sem, sem)

    def issue_last(c, slot):
        sem = kv_sems.at[slot]
        src, dst, rows, piece = v_cp(NHEAD - 1, c, slot)
        if c < NCH - 1:
            _start_pair(*_halves(src, dst, rows, piece), sem, sem)
            return
        pv_ = _pieces(rows, piece)
        pw_ = [(LATE0 + o + oo, nn, u) for u, (o, n) in enumerate(LATE)
               for oo, nn in _pieces(n, C_PIECE)]
        for i in range(max(len(pv_), len(pw_))):
            if i < len(pv_):
                sl = pl.ds(*pv_[i])
                pltpu.make_async_copy(src.at[sl], dst.at[sl], sem).start(priority=0)
            if i < len(pw_):
                sl = pl.ds(pw_[i][0], pw_[i][1])
                pltpu.make_async_copy(bwo_hbm.at[sl], bwo_buf.at[sl],
                                      late_sems.at[pw_[i][2]]).start(priority=1)

    def issue_tick(j, c):
        slot = slot_of(j, c)
        if isinstance(j, int):
            if j == -1:
                sem = kv_sems.at[slot]
                _start_pair(*_halves(*k_cp(0, c, slot)), sem, sem)
            else:
                issue_pair(j, c, slot)
            return

        @pl.when(j < NHEAD - 1)
        def _():
            issue_pair(j, c, slot)

        @pl.when(j == NHEAD - 1)
        def _():
            issue_last(c, slot)

    def issue_next(j, c):
        dj, c2 = divmod(c + NS, NCH)
        issue_tick(j + dj, c2)

    def rows_cp(hbm, buf, start, nrows, piece):
        if not isinstance(start, int):
            start = pl.multiple_of(start, nrows)
        rows = pl.ds(start, nrows)
        return (hbm.at[rows], buf.at[rows], nrows, piece)

    def part_copies(kind, i):
        if kind == 0:
            return (rows_cp(bwq_hbm, bwq_buf, i * WROWS, WROWS, N_PIECE),
                    rows_cp(bwuk_hbm, bwuk_buf, i * WROWS, WROWS, N_PIECE))
        if kind == 1:
            i = i - P_CKV
            return (rows_cp(ckv_hbm, ckv_buf, i * CROWS, CROWS, C_PIECE),
                    rows_cp(ckv_hbm, ckv_buf, SK + i * CROWS, CROWS, C_PIECE))
        if kind == 2:
            i = i - P_UV
            return (rows_cp(bwuv_hbm, bwuv_buf, i * WROWS, WROWS, N_PIECE),
                    rows_cp(bwo_hbm, bwo_buf, i * CROWS, CROWS, C_PIECE))
        return _halves(*rows_cp(bwuv_hbm, bwuv_buf, (P_END - 1 - P_UV) * WROWS, WROWS, N_PIECE))

    def part_do(i, fn):
        sa, sb = b_sems.at[0, i % 4], b_sems.at[1, i % 4]
        if isinstance(i, int):
            fn(*part_copies(0, i), sa, sb)
            return
        for kind, (lo, hi) in enumerate(((0, P_CKV), (P_CKV, P_UV), (P_UV, P_END - 1),
                                         (P_END - 1, P_END))):
            @pl.when((i >= lo) & (i < hi))
            def _():
                fn(*part_copies(kind, i), sa, sb)

    def part_wait(a, b, sa, sb):
        _wait(a[1], sa)
        _wait(b[1], sb)

    x_cp = pltpu.make_async_copy(x_hbm, x_buf, misc_sems.at[0])
    gw_cp = pltpu.make_async_copy(gw_hbm, gw_buf, misc_sems.at[1])
    x_cp.start()
    gw_cp.start()
    i = 0
    for r in range(0, DM, 16):
        for c in range(0, H * DH, 1024):
            sl = (pl.ds(r, 16), pl.ds(c, 1024))
            pltpu.make_async_copy(wq_hbm.at[sl], wq_buf.at[sl], misc_sems.at[2]).start(priority=0)
            sl = pl.ds(i * 32, 32)
            pltpu.make_async_copy(wo_hbm.at[sl], wo_buf.at[sl], misc_sems.at[3]).start(priority=1)
            i += 1
    for t in range(NS):
        issue_tick(t // NCH - 1, t % NCH)
    part_do(0, _start_pair)

    acca_scr[...] = jnp.zeros_like(acca_scr)
    qb_acc[...] = jnp.zeros_like(qb_acc)
    mb_scr[...] = jnp.full_like(mb_scr, -jnp.inf)
    lb_scr[...] = jnp.zeros_like(lb_scr)
    accb_scr[...] = jnp.zeros_like(accb_scr)
    ctx_scr[...] = jnp.zeros_like(ctx_scr)
    outb_scr[...] = jnp.zeros_like(outb_scr)

    x_cp.wait()
    gw_cp.wait()
    x0 = x_buf[0:1, :].astype(F32)
    x1 = x_buf[1:2, :].astype(F32)
    row8 = jax.lax.broadcasted_iota(jnp.int32, (8, DM), 0)

    def rows01(r0, r1, rows):
        return jnp.where(rows == 0, r0, jnp.where(rows == 1, r1, 0.0))

    x8 = rows01(x0, x1, row8)
    x8b = x8.astype(BF16)
    gate = jax.nn.sigmoid(
        jnp.sum(x8 * gw_buf[...].astype(F32).reshape(1, DM), axis=-1, keepdims=True))

    def head_slice(h):
        return pl.ds(h * DH if isinstance(h, int) else pl.multiple_of(h * DH, DH), DH)

    def q_of(h):
        return _dot(x8b, wq_buf[:, head_slice(h)]).astype(BF16)

    def qk(q, c, slot):
        s_scr[:, c * CH:(c + 1) * CH] = _dot_nt(q, ring[slot, 0:CH, :])

    def softmax():
        s = s_scr[...]
        m = jnp.max(s, axis=-1, keepdims=True)
        p = jnp.exp((s - m) * scale)
        p_scr[...] = p.astype(BF16)
        return jnp.sum(p, axis=-1, keepdims=True)

    def pv(c, slot):
        return _dot(p_scr[:, c * CH:(c + 1) * CH], ring[slot, CH:2 * CH, :])

    def finalize(j, acc, l):
        r8 = jax.lax.broadcasted_iota(jnp.int32, (8, DH), 0)
        o = jnp.where(r8 == j // H, acc / l, 0.0).astype(BF16)
        acca_scr[...] += _dot(o, wo_buf[head_slice(j % H), :])

    def phase_wq(j):
        nm = WROWS // H
        base = j * nm

        @pl.when(j == 0)
        def _():
            xcol_scr[0] = jnp.broadcast_to(x0, (128, DM)).T
            xcol_scr[1] = jnp.broadcast_to(x1, (128, DM)).T

        def body(m, carry):
            a0, a1 = carry
            w = bwq_buf[pl.ds(pl.multiple_of((base + m) * H, H), H), :].astype(F32)
            a0 = a0 + w * xcol_scr[0, pl.ds(base + m, 1), :]
            a1 = a1 + w * xcol_scr[1, pl.ds(base + m, 1), :]
            return a0, a1

        a0, a1 = jax.lax.fori_loop(0, nm, body,
                                   (qb_acc[0:H, :], qb_acc[H:2 * H, :]), unroll=8)
        qb_acc[0:H, :] = a0
        qb_acc[H:2 * H, :] = a1

    def phase_uk(j):
        i = j - J_UK
        n = 128 * H
        rows = pl.ds(pl.multiple_of(i * n, n), n)
        qb = qb_acc[...].astype(BF16)
        r = _dot_nt(bwuk_buf[rows, :], qb)
        rr, cc = _iota2((H, 128))
        keep = rr == (cc % H)
        r3 = jnp.where(keep[None], r.reshape(128, H, 128), 0.0)
        qat = jnp.sum(r3, axis=1)
        qabs_scr[i] = qat.T.astype(BF16)

    def phase_ckv(j):
        i = j - J_CKV
        for b in range(B):
            rows = pl.ds(pl.multiple_of(b * SK + i * CROWS, CROWS), CROWS)
            hrows = slice(b * H, (b + 1) * H)
            s = jnp.zeros((H, CROWS), F32)
            for t in range(DC // 128):
                s = s + _dot_nt(qabs_scr[t, hrows, :], ckv_buf[rows, t * 128:(t + 1) * 128])
            m_old = mb_scr[hrows, :]
            m_new = jnp.maximum(m_old, jnp.max(s, axis=-1, keepdims=True))
            alpha = jnp.exp((m_old - m_new) * scale)
            p = jnp.exp((s - m_new) * scale)
            lb_scr[hrows, :] = lb_scr[hrows, :] * alpha + jnp.sum(p, axis=-1, keepdims=True)
            accb_scr[hrows, :] = (accb_scr[hrows, :] * alpha
                                  + _dot(p.astype(BF16), ckv_buf[rows, :]))
            mb_scr[hrows, :] = m_new

    def phase_uv(j):
        i = j - J_UV
        n = 128 * H
        rows = pl.ds(pl.multiple_of(i * n, n), n)

        @pl.when(i == 0)
        def _():
            cc = (accb_scr[...] / lb_scr[...]).astype(BF16)
            for t in range(DC // 128):
                cc_scr[t] = cc[:, t * 128:(t + 1) * 128]
            e_row, e_col = _iota2((128, n))
            e0_scr[...] = jnp.where(e_col // H == e_row, 1.0, 0.0).astype(BF16)

        z = _dot(cc_scr[i], e0_scr[...])
        rr, cc = _iota2((2 * H, n))
        z = jnp.where((rr % H) == (cc % H), z, 0.0).astype(BF16)
        ctx_scr[...] += _dot(z, bwuv_buf[rows, :])

    def wo_lhs(h0, nh):
        lhs = jnp.concatenate([ctx_scr[...]] * nh, axis=1)
        rr, cc = _iota2((2 * H, nh * DH))
        return jnp.where((rr % H) == (cc // DH + h0), lhs, 0.0)

    def phase_wo(j):
        i = j - J_WO
        nh = (LATE0 // DH) // (J_END - J_WO)
        n = nh * DH
        rows = pl.ds(pl.multiple_of(i * n, DH), n)
        outb_scr[...] += _dot(wo_lhs(i * nh, nh).astype(BF16), bwo_buf[rows, :])

    _wait(wq_buf, misc_sems.at[2])
    q0 = q_of(0)
    for c in range(NCH):
        slot = slot_of(-1, c)
        _wait(ring.at[slot, pl.ds(0, CH)], kv_sems.at[slot])
        qk(q0, c, slot)
        issue_next(-1, c)
    l0 = softmax()
    _wait(wo_buf, misc_sems.at[3])

    def head_body(j, l):
        q = q_of((j + 1) % H)
        acc = jnp.zeros((8, DH), F32)
        for c in range(NCH):
            slot = slot_of(j, c)
            _wait(ring.at[slot], kv_sems.at[slot])
            qk(q, c, slot)
            acc = acc + pv(c, slot)
            issue_next(j, c)

        @pl.when(j + 1 < P_END)
        def _():
            part_do(j + 1, _start_pair)

        finalize(j, acc, l)
        l_next = softmax()

        @pl.when(j < P_END)
        def _():
            part_do(j, part_wait)

        for phase, lo, hi in ((phase_wq, 0, J_UK), (phase_uk, J_UK, J_CKV),
                              (phase_ckv, J_CKV, J_CKV + P_UV - P_CKV),
                              (phase_uv, J_UV, J_WO), (phase_wo, J_WO, J_END)):
            @pl.when((j >= lo) & (j < hi))
            def _():
                phase(j)

        return l_next

    l = jax.lax.fori_loop(0, NHEAD - 1, head_body, l0)

    def batch_rows(a):
        rows = jax.lax.broadcasted_iota(jnp.int32, (8, a.shape[1]), 0)
        return rows01(jnp.sum(a[0:H], axis=0, keepdims=True),
                      jnp.sum(a[H:2 * H], axis=0, keepdims=True), rows)

    outb = batch_rows(outb_scr[...])
    lhs8 = batch_rows(wo_lhs(LATE0 // DH, H - LATE0 // DH)).astype(BF16)

    acc = jnp.zeros((8, DH), F32)
    for c in range(NCH):
        slot = slot_of(NHEAD - 1, c)
        _wait(ring.at[slot, pl.ds(CH, CH)], kv_sems.at[slot])
        acc = acc + pv(c, slot)
    finalize(NHEAD - 1, acc, l)
    res = gate * acca_scr[...] + (1.0 - gate) * outb
    late = jnp.zeros((8, DM), F32)
    for u, (o, n) in enumerate(LATE):
        rows = pl.ds(LATE0 + o, n)
        _wait(bwo_buf.at[rows], late_sems.at[u])
        late = late + _dot(lhs8[:, o:o + n], bwo_buf[rows, :])
    res = (res + (1.0 - gate) * late).astype(BF16)
    o_ref[...] = res[0:B]


@jax.jit
def pallas_gated_mix__mha_block_cached__compressed_kv_cla__decode_kernel(
    A_x: jax.Array,
    A_k_cache: jax.Array,
    A_v_cache: jax.Array,
    A_wq: jax.Array,
    A_wo: jax.Array,
    B_x: jax.Array,
    B_c_kv: jax.Array,
    B_w_q: jax.Array,
    B_w_uk: jax.Array,
    B_w_uv: jax.Array,
    B_w_o: jax.Array,
    gate_w: jax.Array,
):
    del B_x
    k = A_k_cache.reshape(NHEAD, SK, DH)
    v = A_v_cache.reshape(NHEAD, SK, DH)
    ckv = B_c_kv.reshape(B * SK, DC)
    bwq = B_w_q.reshape(DM * H, DH)
    bwuk = B_w_uk.reshape(DC * H, DH)
    bwuv = B_w_uv.reshape(DC * H, DH)
    bwo = B_w_o.reshape(H * DH, DM)

    any_spec = pl.BlockSpec(memory_space=pl.ANY)
    scratch = [
        pltpu.VMEM((B, DM), BF16),
        pltpu.VMEM((DM,), BF16),
        pltpu.VMEM((DM, H * DH), BF16),
        pltpu.VMEM((H * DH, DM), BF16),
        pltpu.VMEM((B * SK, DC), BF16),
        pltpu.VMEM((DM * H, DH), BF16),
        pltpu.VMEM((DC * H, DH), BF16),
        pltpu.VMEM((DC * H, DH), BF16),
        pltpu.VMEM((H * DH, DM), BF16),
        pltpu.VMEM((NS, 2 * CH, DH), BF16),
        pltpu.VMEM((8, SK), F32),
        pltpu.VMEM((8, SK), BF16),
        pltpu.VMEM((8, DM), F32),
        pltpu.VMEM((B, DM, 128), F32),
        pltpu.VMEM((128, DH), F32),
        pltpu.VMEM((DC // 128, 128, 128), BF16),
        pltpu.VMEM((2 * H, 1), F32),
        pltpu.VMEM((2 * H, 1), F32),
        pltpu.VMEM((2 * H, DC), F32),
        pltpu.VMEM((DC // 128, 2 * H, 128), BF16),
        pltpu.VMEM((128, 128 * H), BF16),
        pltpu.VMEM((2 * H, DH), F32),
        pltpu.VMEM((2 * H, DM), F32),
        pltpu.SemaphoreType.DMA((NS,)),
        pltpu.SemaphoreType.DMA((2, 4)),
        pltpu.SemaphoreType.DMA((4,)),
        pltpu.SemaphoreType.DMA((len(LATE),)),
    ]
    out = pl.pallas_call(
        _kernel,
        in_specs=[any_spec] * 11,
        out_specs=pl.BlockSpec(memory_space=pltpu.VMEM),
        out_shape=jax.ShapeDtypeStruct((B, DM), BF16),
        scratch_shapes=scratch,
        compiler_params=pltpu.CompilerParams(vmem_limit_bytes=100 * 1024 * 1024,
                                             disable_semaphore_checks=True),
    )(A_x.reshape(B, DM), k, v, A_wq, A_wo, ckv, bwq, bwuk, bwuv, bwo, gate_w)
    return out.reshape(B, 1, DM)
```

```python
import jax
import jax.numpy as jnp
import jax.experimental.pallas as pl
import jax.experimental.pallas.tpu as pltpu

F32 = jnp.float32
BF16 = jnp.bfloat16
_NT = (((1,), (1,)), ((), ()))

B, H, SK, DH, DM = 2, 32, 8192, 128, 512
DC = 4 * DH
NHEAD = B * H
NCH = 4
CH = SK // NCH
NS = 8
N_PIECE = 160
C_PIECE = 40
WROWS = 2048
CROWS = 512
P_CKV, P_UV, P_END = 8, 24, 32
J_UK, J_CKV, J_UV, J_WO, J_END = 8, 12, 32, 36, 40
LATE0 = 28 * DH
LATE = ((0, 256), (256, 128), (384, 128))


def _dot(a, b):
    return jnp.dot(a, b, preferred_element_type=F32)


def _dot_nt(a, b):
    return jax.lax.dot_general(a, b, _NT, preferred_element_type=F32)


def _iota2(shape):
    return (jax.lax.broadcasted_iota(jnp.int32, shape, 0),
            jax.lax.broadcasted_iota(jnp.int32, shape, 1))


def _pieces(rows, piece):
    return [(o, min(piece, rows - o)) for o in range(0, rows, piece)]


def _start_pair(a, b, sem_a, sem_b):
    pa, pb = _pieces(a[2], a[3]), _pieces(b[2], b[3])
    for i in range(max(len(pa), len(pb))):
        for t, (cp, ps, sem) in enumerate(((a, pa, sem_a), (b, pb, sem_b))):
            if i < len(ps):
                sl = pl.ds(*ps[i])
                pltpu.make_async_copy(cp[0].at[sl], cp[1].at[sl], sem).start(priority=t)


def _halves(src, dst, rows, piece):
    half = rows // 2
    lo, hi = pl.ds(0, half), pl.ds(half, half)
    return ((src.at[lo], dst.at[lo], half, piece), (src.at[hi], dst.at[hi], half, piece))


def _wait(dst, sem):
    pltpu.make_async_copy(dst, dst, sem).wait()


def _kernel(x_hbm, k_hbm, v_hbm, wq_hbm, wo_hbm, ckv_hbm, bwq_hbm, bwuk_hbm,
            bwuv_hbm, bwo_hbm, gw_hbm, o_ref,
            x_buf, gw_buf, wq_buf, wo_buf, ckv_buf, bwq_buf, bwuk_buf,
            bwuv_buf, bwo_buf, ring,
            s_scr, p_scr, acca_scr, xcol_scr, qb_acc, qabs_scr,
            mb_scr, lb_scr, accb_scr, cc_scr, e0_scr, ctx_scr, outb_scr,
            kv_sems, b_sems, misc_sems, late_sems):
    scale = DH ** -0.5

    def slot_of(j, c):
        return (NCH * (j + 1) + c) % NS

    def k_cp(j, c, slot):
        return (k_hbm.at[j, pl.ds(c * CH, CH)], ring.at[slot, pl.ds(0, CH)], CH, N_PIECE)

    def v_cp(j, c, slot):
        return (v_hbm.at[j, pl.ds(c * CH, CH)], ring.at[slot, pl.ds(CH, CH)], CH, N_PIECE)

    def issue_pair(j, c, slot):
        sem = kv_sems.at[slot]
        _start_pair(k_cp(j + 1, c, slot), v_cp(j, c, slot), sem, sem)

    def issue_last(c, slot):
        sem = kv_sems.at[slot]
        src, dst, rows, piece = v_cp(NHEAD - 1, c, slot)
        if c < NCH - 1:
            _start_pair(*_halves(src, dst, rows, piece), sem, sem)
            return
        pv_ = _pieces(rows, piece)
        pw_ = [(LATE0 + o + oo, nn, u) for u, (o, n) in enumerate(LATE)
               for oo, nn in _pieces(n, C_PIECE)]
        for i in range(max(len(pv_), len(pw_))):
            if i < len(pv_):
                sl = pl.ds(*pv_[i])
                pltpu.make_async_copy(src.at[sl], dst.at[sl], sem).start(priority=0)
            if i < len(pw_):
                sl = pl.ds(pw_[i][0], pw_[i][1])
                pltpu.make_async_copy(bwo_hbm.at[sl], bwo_buf.at[sl],
                                      late_sems.at[pw_[i][2]]).start(priority=1)

    def issue_tick(j, c):
        slot = slot_of(j, c)
        if isinstance(j, int):
            if j == -1:
                sem = kv_sems.at[slot]
                _start_pair(*_halves(*k_cp(0, c, slot)), sem, sem)
            else:
                issue_pair(j, c, slot)
            return

        @pl.when(j < NHEAD - 1)
        def _():
            issue_pair(j, c, slot)

        @pl.when(j == NHEAD - 1)
        def _():
            issue_last(c, slot)

    def issue_next(j, c):
        dj, c2 = divmod(c + NS, NCH)
        issue_tick(j + dj, c2)

    def rows_cp(hbm, buf, start, nrows, piece):
        if not isinstance(start, int):
            start = pl.multiple_of(start, nrows)
        rows = pl.ds(start, nrows)
        return (hbm.at[rows], buf.at[rows], nrows, piece)

    def part_copies(kind, i):
        if kind == 0:
            return (rows_cp(bwq_hbm, bwq_buf, i * WROWS, WROWS, N_PIECE),
                    rows_cp(bwuk_hbm, bwuk_buf, i * WROWS, WROWS, N_PIECE))
        if kind == 1:
            i = i - P_CKV
            return (rows_cp(ckv_hbm, ckv_buf, i * CROWS, CROWS, C_PIECE),
                    rows_cp(ckv_hbm, ckv_buf, SK + i * CROWS, CROWS, C_PIECE))
        if kind == 2:
            i = i - P_UV
            return (rows_cp(bwuv_hbm, bwuv_buf, i * WROWS, WROWS, N_PIECE),
                    rows_cp(bwo_hbm, bwo_buf, i * CROWS, CROWS, C_PIECE))
        return _halves(*rows_cp(bwuv_hbm, bwuv_buf, (P_END - 1 - P_UV) * WROWS, WROWS, N_PIECE))

    def part_do(i, fn):
        sa, sb = b_sems.at[0, i % 4], b_sems.at[1, i % 4]
        if isinstance(i, int):
            fn(*part_copies(0, i), sa, sb)
            return
        for kind, (lo, hi) in enumerate(((0, P_CKV), (P_CKV, P_UV), (P_UV, P_END - 1),
                                         (P_END - 1, P_END))):
            @pl.when((i >= lo) & (i < hi))
            def _():
                fn(*part_copies(kind, i), sa, sb)

    def part_wait(a, b, sa, sb):
        _wait(a[1], sa)
        _wait(b[1], sb)

    x_cp = pltpu.make_async_copy(x_hbm, x_buf, misc_sems.at[0])
    gw_cp = pltpu.make_async_copy(gw_hbm, gw_buf, misc_sems.at[1])
    x_cp.start()
    gw_cp.start()
    i = 0
    for r in range(0, DM, 16):
        for c in range(0, H * DH, 1024):
            sl = (pl.ds(r, 16), pl.ds(c, 1024))
            pltpu.make_async_copy(wq_hbm.at[sl], wq_buf.at[sl], misc_sems.at[2]).start(priority=0)
            sl = pl.ds(i * 32, 32)
            pltpu.make_async_copy(wo_hbm.at[sl], wo_buf.at[sl], misc_sems.at[3]).start(priority=1)
            i += 1
    for t in range(NS):
        issue_tick(t // NCH - 1, t % NCH)
    part_do(0, _start_pair)

    acca_scr[...] = jnp.zeros_like(acca_scr)
    qb_acc[...] = jnp.zeros_like(qb_acc)
    mb_scr[...] = jnp.full_like(mb_scr, -jnp.inf)
    lb_scr[...] = jnp.zeros_like(lb_scr)
    accb_scr[...] = jnp.zeros_like(accb_scr)
    ctx_scr[...] = jnp.zeros_like(ctx_scr)
    outb_scr[...] = jnp.zeros_like(outb_scr)

    x_cp.wait()
    gw_cp.wait()
    x0 = x_buf[0:1, :].astype(F32)
    x1 = x_buf[1:2, :].astype(F32)
    row8 = jax.lax.broadcasted_iota(jnp.int32, (8, DM), 0)

    def rows01(r0, r1, rows):
        return jnp.where(rows == 0, r0, jnp.where(rows == 1, r1, 0.0))

    x8 = rows01(x0, x1, row8)
    x8b = x8.astype(BF16)
    gate = jax.nn.sigmoid(
        jnp.sum(x8 * gw_buf[...].astype(F32).reshape(1, DM), axis=-1, keepdims=True))

    def head_slice(h):
        return pl.ds(h * DH if isinstance(h, int) else pl.multiple_of(h * DH, DH), DH)

    def q_of(h):
        return _dot(x8b, wq_buf[:, head_slice(h)]).astype(BF16)

    def qk(q, c, slot):
        s_scr[:, c * CH:(c + 1) * CH] = _dot_nt(q, ring[slot, 0:CH, :])

    def softmax():
        s = s_scr[...]
        m = jnp.max(s, axis=-1, keepdims=True)
        p = jnp.exp((s - m) * scale)
        p_scr[...] = p.astype(BF16)
        return jnp.sum(p, axis=-1, keepdims=True)

    def pv(c, slot):
        return _dot(p_scr[:, c * CH:(c + 1) * CH], ring[slot, CH:2 * CH, :])

    def finalize(j, acc, l):
        r8 = jax.lax.broadcasted_iota(jnp.int32, (8, DH), 0)
        o = jnp.where(r8 == j // H, acc / l, 0.0).astype(BF16)
        acca_scr[...] += _dot(o, wo_buf[head_slice(j % H), :])

    def phase_wq(j):
        nm = WROWS // H
        base = j * nm

        @pl.when(j == 0)
        def _():
            xcol_scr[0] = jnp.broadcast_to(x0, (128, DM)).T
            xcol_scr[1] = jnp.broadcast_to(x1, (128, DM)).T

        def body(m, carry):
            a0, a1 = carry
            w = bwq_buf[pl.ds(pl.multiple_of((base + m) * H, H), H), :].astype(F32)
            a0 = a0 + w * xcol_scr[0, pl.ds(base + m, 1), :]
            a1 = a1 + w * xcol_scr[1, pl.ds(base + m, 1), :]
            return a0, a1

        a0, a1 = jax.lax.fori_loop(0, nm, body,
                                   (qb_acc[0:H, :], qb_acc[H:2 * H, :]), unroll=8)
        qb_acc[0:H, :] = a0
        qb_acc[H:2 * H, :] = a1

    def phase_uk(j):
        i = j - J_UK
        n = 128 * H
        rows = pl.ds(pl.multiple_of(i * n, n), n)
        qb = qb_acc[...].astype(BF16)
        r = _dot_nt(bwuk_buf[rows, :], qb)
        rr, cc = _iota2((H, 128))
        keep = rr == (cc % H)
        r3 = jnp.where(keep[None], r.reshape(128, H, 128), 0.0)
        qat = jnp.sum(r3, axis=1)
        qabs_scr[i] = qat.T.astype(BF16)

    def phase_ckv(j):
        i = j - J_CKV
        for b in range(B):
            rows = pl.ds(pl.multiple_of(b * SK + i * CROWS, CROWS), CROWS)
            hrows = slice(b * H, (b + 1) * H)
            s = jnp.zeros((H, CROWS), F32)
            for t in range(DC // 128):
                s = s + _dot_nt(qabs_scr[t, hrows, :], ckv_buf[rows, t * 128:(t + 1) * 128])
            m_old = mb_scr[hrows, :]
            m_new = jnp.maximum(m_old, jnp.max(s, axis=-1, keepdims=True))
            alpha = jnp.exp((m_old - m_new) * scale)
            p = jnp.exp((s - m_new) * scale)
            lb_scr[hrows, :] = lb_scr[hrows, :] * alpha + jnp.sum(p, axis=-1, keepdims=True)
            accb_scr[hrows, :] = (accb_scr[hrows, :] * alpha
                                  + _dot(p.astype(BF16), ckv_buf[rows, :]))
            mb_scr[hrows, :] = m_new

    def phase_uv(j):
        i = j - J_UV
        n = 128 * H
        rows = pl.ds(pl.multiple_of(i * n, n), n)

        @pl.when(i == 0)
        def _():
            cc = (accb_scr[...] / lb_scr[...]).astype(BF16)
            for t in range(DC // 128):
                cc_scr[t] = cc[:, t * 128:(t + 1) * 128]
            e_row, e_col = _iota2((128, n))
            e0_scr[...] = jnp.where(e_col // H == e_row, 1.0, 0.0).astype(BF16)

        z = _dot(cc_scr[i], e0_scr[...])
        rr, cc = _iota2((2 * H, n))
        z = jnp.where((rr % H) == (cc % H), z, 0.0).astype(BF16)
        ctx_scr[...] += _dot(z, bwuv_buf[rows, :])

    def wo_lhs(h0, nh):
        lhs = jnp.concatenate([ctx_scr[...]] * nh, axis=1)
        rr, cc = _iota2((2 * H, nh * DH))
        return jnp.where((rr % H) == (cc // DH + h0), lhs, 0.0)

    def phase_wo(j):
        i = j - J_WO
        nh = (LATE0 // DH) // (J_END - J_WO)
        n = nh * DH
        rows = pl.ds(pl.multiple_of(i * n, DH), n)
        outb_scr[...] += _dot(wo_lhs(i * nh, nh).astype(BF16), bwo_buf[rows, :])

    _wait(wq_buf, misc_sems.at[2])
    q0 = q_of(0)
    for c in range(NCH):
        slot = slot_of(-1, c)
        _wait(ring.at[slot, pl.ds(0, CH)], kv_sems.at[slot])
        qk(q0, c, slot)
        issue_next(-1, c)
    l0 = softmax()
    _wait(wo_buf, misc_sems.at[3])

    def head_body(j, l):
        q = q_of((j + 1) % H)
        acc = jnp.zeros((8, DH), F32)
        for c in range(NCH):
            slot = slot_of(j, c)
            _wait(ring.at[slot], kv_sems.at[slot])
            qk(q, c, slot)
            acc = acc + pv(c, slot)
            issue_next(j, c)

        @pl.when(j + 1 < P_END)
        def _():
            part_do(j + 1, _start_pair)

        finalize(j, acc, l)
        l_next = softmax()

        @pl.when(j < P_END)
        def _():
            part_do(j, part_wait)

        for phase, lo, hi in ((phase_wq, 0, J_UK), (phase_uk, J_UK, J_CKV),
                              (phase_ckv, J_CKV, J_CKV + P_UV - P_CKV),
                              (phase_uv, J_UV, J_WO), (phase_wo, J_WO, J_END)):
            @pl.when((j >= lo) & (j < hi))
            def _():
                phase(j)

        return l_next

    l = jax.lax.fori_loop(0, NHEAD - 1, head_body, l0)

    def batch_rows(a):
        rows = jax.lax.broadcasted_iota(jnp.int32, (8, a.shape[1]), 0)
        return rows01(jnp.sum(a[0:H], axis=0, keepdims=True),
                      jnp.sum(a[H:2 * H], axis=0, keepdims=True), rows)

    outb = batch_rows(outb_scr[...])
    lhs8 = batch_rows(wo_lhs(LATE0 // DH, H - LATE0 // DH)).astype(BF16)

    acc = jnp.zeros((8, DH), F32)
    for c in range(NCH):
        slot = slot_of(NHEAD - 1, c)
        _wait(ring.at[slot, pl.ds(CH, CH)], kv_sems.at[slot])
        acc = acc + pv(c, slot)
    finalize(NHEAD - 1, acc, l)
    res = gate * acca_scr[...] + (1.0 - gate) * outb
    late = jnp.zeros((8, DM), F32)
    for u, (o, n) in enumerate(LATE):
        rows = pl.ds(LATE0 + o, n)
        _wait(bwo_buf.at[rows], late_sems.at[u])
        late = late + _dot(lhs8[:, o:o + n], bwo_buf[rows, :])
    res = (res + (1.0 - gate) * late).astype(BF16)
    o_ref[...] = res[0:B]


def _compiler_params():
    limit = 100 * 1024 * 1024
    try:
        return pltpu.CompilerParams(vmem_limit_bytes=limit, disable_semaphore_checks=True)
    except TypeError:
        return pltpu.CompilerParams(vmem_limit_bytes=limit)


@jax.jit
def pallas_gated_mix__mha_block_cached__compressed_kv_cla__decode_kernel(
    A_x: jax.Array,
    A_k_cache: jax.Array,
    A_v_cache: jax.Array,
    A_wq: jax.Array,
    A_wo: jax.Array,
    B_x: jax.Array,
    B_c_kv: jax.Array,
    B_w_q: jax.Array,
    B_w_uk: jax.Array,
    B_w_uv: jax.Array,
    B_w_o: jax.Array,
    gate_w: jax.Array,
):
    del B_x
    k = A_k_cache.reshape(NHEAD, SK, DH)
    v = A_v_cache.reshape(NHEAD, SK, DH)
    ckv = B_c_kv.reshape(B * SK, DC)
    bwq = B_w_q.reshape(DM * H, DH)
    bwuk = B_w_uk.reshape(DC * H, DH)
    bwuv = B_w_uv.reshape(DC * H, DH)
    bwo = B_w_o.reshape(H * DH, DM)

    any_spec = pl.BlockSpec(memory_space=pl.ANY)
    scratch = [
        pltpu.VMEM((B, DM), BF16),
        pltpu.VMEM((DM,), BF16),
        pltpu.VMEM((DM, H * DH), BF16),
        pltpu.VMEM((H * DH, DM), BF16),
        pltpu.VMEM((B * SK, DC), BF16),
        pltpu.VMEM((DM * H, DH), BF16),
        pltpu.VMEM((DC * H, DH), BF16),
        pltpu.VMEM((DC * H, DH), BF16),
        pltpu.VMEM((H * DH, DM), BF16),
        pltpu.VMEM((NS, 2 * CH, DH), BF16),
        pltpu.VMEM((8, SK), F32),
        pltpu.VMEM((8, SK), BF16),
        pltpu.VMEM((8, DM), F32),
        pltpu.VMEM((B, DM, 128), F32),
        pltpu.VMEM((128, DH), F32),
        pltpu.VMEM((DC // 128, 128, 128), BF16),
        pltpu.VMEM((2 * H, 1), F32),
        pltpu.VMEM((2 * H, 1), F32),
        pltpu.VMEM((2 * H, DC), F32),
        pltpu.VMEM((DC // 128, 2 * H, 128), BF16),
        pltpu.VMEM((128, 128 * H), BF16),
        pltpu.VMEM((2 * H, DH), F32),
        pltpu.VMEM((2 * H, DM), F32),
        pltpu.SemaphoreType.DMA((NS,)),
        pltpu.SemaphoreType.DMA((2, 4)),
        pltpu.SemaphoreType.DMA((4,)),
        pltpu.SemaphoreType.DMA((len(LATE),)),
    ]
    out = pl.pallas_call(
        _kernel,
        in_specs=[any_spec] * 11,
        out_specs=pl.BlockSpec(memory_space=pltpu.VMEM),
        out_shape=jax.ShapeDtypeStruct((B, DM), BF16),
        scratch_shapes=scratch,
        compiler_params=_compiler_params(),
    )(A_x.reshape(B, DM), k, v, A_wq, A_wo, ckv, bwq, bwuk, bwuv, bwo, gate_w)
    return out.reshape(B, 1, DM)
```
